```python
import os as _os
_os.environ.setdefault('JAX_PLATFORMS', 'cpu')
import jax
import jax.numpy as jnp

def _softmax(x, axis=-1):
    return jax.nn.softmax(x, axis=axis)

def _gelu(x):
    return jax.nn.gelu(x, approximate=True)

def _silu(x):
    return jax.nn.silu(x)

def _sigmoid(x):
    return jax.nn.sigmoid(x)

def _layernorm(x, axis=-1, eps=1e-05):
    m = jnp.mean(x, axis=axis, keepdims=True)
    v = jnp.var(x, axis=axis, keepdims=True)
    return (x - m) / jnp.sqrt(v + eps)

def _scatter_add(tgt, idx, src, axis=0):
    return tgt.at[idx].add(src)

def _segment_sum(src, seg, n):
    return jax.ops.segment_sum(src, seg, n)

class _Rng:

    def __init__(self, key):
        self._k = key

    def _next(self):
        self._k, sub = jax.random.split(self._k)
        return sub

    def normal(self, shape):
        return jax.random.normal(self._next(), shape, dtype=jnp.bfloat16)

    def randint(self, lo, hi, shape):
        return jax.random.randint(self._next(), shape, lo, hi, dtype=jnp.int32)

    def uniform(self, shape, lo=0.0, hi=1.0):
        return jax.random.uniform(self._next(), shape, jnp.bfloat16, lo, hi)

    def permutation(self, n):
        return jax.random.permutation(self._next(), n)
kernel_name = 'adaLN_cond__mha_block_cached__geglu_ffn__prompt'

def setup_inputs():
    _rng = _Rng(jax.random.key(int.from_bytes(__import__("os").urandom(4), "little")))
    _w = lambda a: (lambda t: t.astype(jnp.bfloat16) if jnp.issubdtype(t.dtype, jnp.floating) else t)(jnp.asarray(a))

    def _A_setup():
        B, Sq, D = (1, 2048, 512)
        H, Sk, Dh = (32, 2048, 128)
        return {'x': _w((lambda *s: _rng.normal(s) * 0.05)(B, Sq, D)), 'k_cache': _w((lambda *s: _rng.normal(s) * 3.2)(B, H, Sk, Dh)), 'v_cache': _w((lambda *s: _rng.normal(s) * 0.4)(B, H, Sk, Dh)), 'wq': _w((lambda *s: _rng.normal(s) * 1.6)(D, H * Dh) * D ** (-0.5)), 'wo': _w((lambda *s: _rng.normal(s) * 0.4)(H * Dh, D) * (H * Dh) ** (-0.5))}
    _A_in = _A_setup()

    def _B_setup():
        B, S, D, F = (1, 2048, 512, 1792)
        return {'x': _w((lambda *s: _rng.normal(s) * 0.05)(B, S, D)), 'w_gate': _w((lambda *s: _rng.normal(s) * 0.05)(D, F)), 'w_up': _w((lambda *s: _rng.normal(s) * 0.05)(D, F)), 'w_down': _w((lambda *s: _rng.normal(s) * 0.05)(F, D))}
    _B_in = _B_setup()
    return {'A_x': _A_in['x'], 'A_k_cache': _A_in['k_cache'], 'A_v_cache': _A_in['v_cache'], 'A_wq': _A_in['wq'], 'A_wo': _A_in['wo'], 'B_x': _B_in['x'], 'B_w_gate': _B_in['w_gate'], 'B_w_up': _B_in['w_up'], 'B_w_down': _B_in['w_down'], 'c': _w((lambda *s: _rng.normal(s) * 0.05)(1, 512) * 8.0), 'w_mod': _w((lambda *s: _rng.normal(s) * 0.05)(512, 6 * 512) * 512 ** (-0.5) * 8.0)}

def reference(A_x, A_k_cache, A_v_cache, A_wq, A_wo, B_x, B_w_gate, B_w_up, B_w_down, c, w_mod):

    def _A_ref(x, k_cache, v_cache, wq, wo):
        B, Sq, D = x.shape
        H, Dh = (32, 128)
        q = (lambda x, *d: x.transpose(*d))((x @ wq).reshape(B, Sq, H, Dh), 0, 2, 1, 3)
        scores = jnp.einsum('bhqd,bhkd->bhqk', q, k_cache) * Dh ** (-0.5)
        p = _softmax(scores, axis=-1)
        o = jnp.einsum('bhqk,bhkd->bhqd', p, v_cache)
        return (lambda x, *d: x.transpose(*d))(o, 0, 2, 1, 3).reshape(B, Sq, H * Dh) @ wo

    def _B_ref(x, w_gate, w_up, w_down):
        return _gelu(x @ w_gate) * (x @ w_up) @ w_down
    x = A_x
    mod = (_silu(c) @ w_mod).reshape(c.shape[0], 6, 1, -1)
    sa, ca, ga, sb, cb, gb = (mod[:, 0].copy(), mod[:, 1].copy(), mod[:, 2].copy(), mod[:, 3].copy(), mod[:, 4].copy(), mod[:, 5].copy())
    h = _layernorm(x, axis=-1) * (1 + ca) + sa
    x = x + ga * _A_ref(h, A_k_cache, A_v_cache, A_wq, A_wo)
    h = _layernorm(x, axis=-1) * (1 + cb) + sb
    x = x + gb * _B_ref(h, B_w_gate, B_w_up, B_w_down)
    return x
```

```python
import math
import numpy as np
import jax
import jax.numpy as jnp
import jax.experimental.pallas as pl
import jax.experimental.pallas.tpu as pltpu

LOG2E = 1.4426950408889634
BQ = 128
AHEAD = 1
FFN_BM = 256


def _ln(xf, eps=1e-5):
    m = jnp.mean(xf, axis=-1, keepdims=True)
    d = xf - m
    v = jnp.mean(d * d, axis=-1, keepdims=True)
    return d * jax.lax.rsqrt(v + eps)


def _gelu(x):
    c = math.sqrt(2.0 / math.pi)
    return 0.5 * x * (1.0 + jnp.tanh(c * (x + 0.044715 * (x * x * x))))


def _dot_t(a, b):
    return jax.lax.dot_general(a, b, (((1,), (1,)), ((), ())), preferred_element_type=jnp.float32)


def _tree(vals, op):
    vals = list(vals)
    while len(vals) > 1:
        nxt = [op(vals[i], vals[i + 1]) for i in range(0, len(vals) - 1, 2)]
        if len(vals) % 2:
            nxt.append(vals[-1])
        vals = nxt
    return vals[0]


def _kernel(z_ref, x_ref, k_ref, v_ref, wq_ref, wo_ref, wg_ref, wu_ref, wd_ref, c_ref, wmod_ref,
            o_ref, h_scr, mod_scr, acc_scr, q_scr, vt_scr, o_scr, *sbs):
    hd = pl.program_id(0)
    S, D = x_ref.shape
    Sk, Dh = k_ref.shape
    bq = BQ
    nu = S // bq

    @pl.when(hd == 0)
    def _():
        c = c_ref[...].astype(jnp.float32)
        sc = c * jax.nn.sigmoid(c)
        scb = jnp.broadcast_to(sc, (16, D)).astype(jnp.bfloat16)
        mod = jnp.dot(scb, wmod_ref[...], preferred_element_type=jnp.float32)
        mod_scr[...] = mod[0:8]
        sa = mod_scr[0:1, 0:D]
        ca = mod_scr[0:1, D:2 * D]

        def body(i, carry):
            r = pl.ds(pl.multiple_of(i * 256, 256), 256)
            xf = x_ref[r, :].astype(jnp.float32)
            h_scr[r, :] = (_ln(xf) * (1.0 + ca) + sa).astype(jnp.bfloat16)
            return carry
        jax.lax.fori_loop(0, S // 256, body, 0)
        acc_scr[...] = jnp.zeros_like(acc_scr)

    scale = Dh ** -0.5 * LOG2E
    ztk = pl.multiple_of(z_ref[0], 8)
    sb = lambda u, g: sbs[(u % 2) * 4 + g]

    vt_scr[...] = v_ref[...].T
    for i in range(S // 256):
        r = slice(i * 256, (i + 1) * 256)
        q = jnp.dot(h_scr[r, :], wq_ref[...], preferred_element_type=jnp.float32)
        q_scr[r, :] = (q * scale).astype(jnp.bfloat16)

    def red(x, op):
        n = x.shape[0] // 8
        return _tree([x[8 * i:8 * (i + 1), :] for i in range(n)], op)

    mx, atok, ls, accs = {}, {}, {}, {}

    def a_chunk(n):
        u, c = divmod(n, 4)
        if u >= nu:
            return
        qt = q_scr[u * bq:(u + 1) * bq, :]
        parts = []
        for m in range(4):
            r0 = 512 * c + 128 * m
            s = _dot_t(k_ref[r0:r0 + 128, :], qt)
            sb(u, c)[128 * m:128 * (m + 1), :] = s
            if m == 3:
                atok[n] = s[0:8, :]
            parts.append(red(s, jnp.maximum))
        sm = _tree(parts, jnp.maximum)
        mx[u] = sm if c == 0 else jnp.maximum(mx[u], sm)
        if c == 3:
            mx[u] = jnp.max(mx[u], axis=0, keepdims=True)

    def exp_group(n):
        u, g = divmod(n, 4)
        if u >= nu:
            return None
        t = atok.get(n + 3)
        if t is None:
            t = atok[max(atok)]
        sb(u, g)[pl.ds(ztk + 512, 8), :] = t
        s = sb(u, g)[0:512, :]
        p = jnp.exp2(s - mx[u])
        ps = red(p, jnp.add)
        ls[u] = ps if g == 0 else ls[u] + ps
        return p.astype(jnp.bfloat16)

    def pv(n, pb):
        u, g = divmod(n, 4)
        o = jnp.dot(vt_scr[:, 512 * g:512 * (g + 1)], pb, preferred_element_type=jnp.float32)
        accs[u] = o if g == 0 else accs[u] + o
        if g == 3:
            lsum = jnp.sum(ls[u], axis=0, keepdims=True)
            o = accs[u] * (1.0 / lsum)
            o_scr[u * bq:(u + 1) * bq, :] = o.T.astype(jnp.bfloat16)

    for n in range(4 + AHEAD):
        a_chunk(n)
    pcur = exp_group(0)
    for n in range(4 * nu):
        pnext = exp_group(n + 1)
        a_chunk(n + 4 + AHEAD)
        pv(n, pcur)
        pcur = pnext
    for i in range(S // 256):
        r = slice(i * 256, (i + 1) * 256)
        acc_scr[r, :] += jnp.dot(o_scr[r, :], wo_ref[...], preferred_element_type=jnp.float32)

    @pl.when(hd == pl.num_programs(0) - 1)
    def _():
        ga = mod_scr[0:1, 2 * D:3 * D]
        sbb = mod_scr[0:1, 3 * D:4 * D]
        cb = mod_scr[0:1, 4 * D:5 * D]
        gb = mod_scr[0:1, 5 * D:6 * D]

        def body(i, carry):
            r = pl.ds(pl.multiple_of(i * FFN_BM, FFN_BM), FFN_BM)
            x1 = x_ref[r, :].astype(jnp.float32) + ga * acc_scr[r, :]
            h = (_ln(x1) * (1.0 + cb) + sbb).astype(jnp.bfloat16)
            g = jnp.dot(h, wg_ref[...], preferred_element_type=jnp.float32)
            u = jnp.dot(h, wu_ref[...], preferred_element_type=jnp.float32)
            a = (_gelu(g) * u).astype(jnp.bfloat16)
            y = jnp.dot(a, wd_ref[...], preferred_element_type=jnp.float32)
            o_ref[r, :] = (x1 + gb * y).astype(o_ref.dtype)
            return carry
        jax.lax.fori_loop(0, S // FFN_BM, body, 0)


@jax.jit
def pallas_adaLN_cond__mha_block_cached__geglu_ffn__prompt_kernel(
    A_x, A_k_cache, A_v_cache, A_wq, A_wo, B_x, B_w_gate, B_w_up, B_w_down, c, w_mod,
):
    B, S, D = A_x.shape
    _, H, Sk, Dh = A_k_cache.shape
    F = B_w_gate.shape[1]
    x = A_x.reshape(S, D)
    k = A_k_cache.reshape(H, Sk, Dh)
    v = A_v_cache.reshape(H, Sk, Dh)
    z = jnp.asarray(np.zeros((8,), np.int32))
    full = lambda shape: pl.BlockSpec(shape, lambda h: (0,) * len(shape))
    out = pl.pallas_call(
        _kernel,
        grid=(H,),
        in_specs=[
            pl.BlockSpec(memory_space=pltpu.SMEM),
            full((S, D)),
            pl.BlockSpec((None, Sk, Dh), lambda h: (h, 0, 0)),
            pl.BlockSpec((None, Sk, Dh), lambda h: (h, 0, 0)),
            pl.BlockSpec((D, Dh), lambda h: (0, h)),
            pl.BlockSpec((Dh, D), lambda h: (h, 0)),
            full((D, F)), full((D, F)), full((F, D)),
            full((1, D)), full((D, 6 * D)),
        ],
        out_specs=full((S, D)),
        out_shape=jax.ShapeDtypeStruct((S, D), jnp.bfloat16),
        scratch_shapes=[
            pltpu.VMEM((S, D), jnp.bfloat16),
            pltpu.VMEM((8, 6 * D), jnp.float32),
            pltpu.VMEM((S, D), jnp.float32),
            pltpu.VMEM((S, Dh), jnp.bfloat16),
            pltpu.VMEM((Dh, Sk), jnp.bfloat16),
            pltpu.VMEM((S, Dh), jnp.bfloat16),
        ] + [pltpu.VMEM((520, BQ), jnp.float32) for _ in range(8)],
        compiler_params=pltpu.CompilerParams(
            dimension_semantics=("arbitrary",),
            vmem_limit_bytes=100 * 1024 * 1024,
        ),
    )(z, x, k, v, A_wq, A_wo, B_w_gate, B_w_up, B_w_down, c, w_mod)
    return out.reshape(B, S, D)
```

```python
import math
import numpy as np
import jax
import jax.numpy as jnp
import jax.experimental.pallas as pl
import jax.experimental.pallas.tpu as pltpu

LOG2E = 1.4426950408889634


def _ln(xf, eps=1e-5):
    m = jnp.mean(xf, axis=-1, keepdims=True)
    d = xf - m
    v = jnp.mean(d * d, axis=-1, keepdims=True)
    return d * jax.lax.rsqrt(v + eps)


def _gelu(x):
    c = math.sqrt(2.0 / math.pi)
    return 0.5 * x * (1.0 + jnp.tanh(c * (x + 0.044715 * (x * x * x))))


def _dot_t(a, b):
    return jax.lax.dot_general(a, b, (((1,), (1,)), ((), ())), preferred_element_type=jnp.float32)


def _tree(vals, op):
    vals = list(vals)
    while len(vals) > 1:
        nxt = [op(vals[i], vals[i + 1]) for i in range(0, len(vals) - 1, 2)]
        if len(vals) % 2:
            nxt.append(vals[-1])
        vals = nxt
    return vals[0]


def _make(flags=None, ffn_bm=256, nh=None, qstep=0, ostep=4, tok_row=64, defer_finish=True, order='jeap', ah=5):
    bq = 128
    AH = ah

    def kernel(z_ref, c_ref, x_hbm, k_hbm, v_hbm, wq_hbm, wo_hbm, wg_hbm, wu_hbm, wd_hbm, wmod_hbm,
               out_hbm,
               x_v, h_scr, mod_scr, acc_scr, q_scr, vt_scr, o_scr, p_scr, carry_scr, oacc_scr,
               k_v, v_v, wq_v, wo_v, wg_v, wu_v, wd_v, wm_v, out_v,
               sem_k, sem_v, sem_wq, sem_wo, sem_x, sem_m, sem_f, sem_o,
               *sbs):
        S, D = x_v.shape
        H = k_hbm.shape[0]
        NH = nh or H
        Sk, Dh = k_v.shape[1:]
        nu = S // bq
        NS = 4 * nu
        XC = 256
        nxc = S // XC

        def k_copy(hsrc, slot):
            return pltpu.make_async_copy(k_hbm.at[jnp.minimum(hsrc, H - 1)], k_v.at[slot], sem_k.at[slot])

        def v_copy(hsrc, slot):
            return pltpu.make_async_copy(v_hbm.at[jnp.minimum(hsrc, H - 1)], v_v.at[slot], sem_v.at[slot])

        def wq_copy(hsrc, slot):
            hs = pl.multiple_of(jnp.minimum(hsrc, H - 1) * Dh, Dh)
            return pltpu.make_async_copy(wq_hbm.at[:, pl.ds(hs, Dh)], wq_v.at[slot], sem_wq.at[slot])

        def wo_copy(hsrc, slot):
            hs = pl.multiple_of(jnp.minimum(hsrc, H - 1) * Dh, Dh)
            return pltpu.make_async_copy(wo_hbm.at[pl.ds(hs, Dh), :], wo_v.at[slot], sem_wo.at[slot])

        def x_copy(i):
            return pltpu.make_async_copy(x_hbm.at[pl.ds(i * XC, XC), :], x_v.at[pl.ds(i * XC, XC), :], sem_x.at[i])

        wm1_copy = pltpu.make_async_copy(wmod_hbm.at[:, pl.ds(0, 2 * D)], wm_v.at[:, pl.ds(0, 2 * D)], sem_m.at[0])
        wm2_copy = pltpu.make_async_copy(wmod_hbm.at[:, pl.ds(2 * D, 4 * D)], wm_v.at[:, pl.ds(2 * D, 4 * D)], sem_m.at[1])
        wg_copy = pltpu.make_async_copy(wg_hbm, wg_v, sem_f.at[0])
        wu_copy = pltpu.make_async_copy(wu_hbm, wu_v, sem_f.at[1])
        wd_copy = pltpu.make_async_copy(wd_hbm, wd_v, sem_f.at[2])

        def out_copy(i):
            r = pl.ds(pl.multiple_of(i * ffn_bm, ffn_bm), ffn_bm)
            return pltpu.make_async_copy(out_v.at[r, :], out_hbm.at[r, :], sem_o.at[i])

        wm1_copy.start()
        for i in range(nxc):
            x_copy(i).start()
        wq_copy(0, 0).start()
        k_copy(0, 0).start()
        v_copy(0, 0).start()
        k_copy(1, 1).start()
        wq_copy(1, 1).start()
        wo_copy(0, 0).start()

        acc_scr[...] = jnp.zeros_like(acc_scr)
        wo_v[2] = jnp.zeros((Dh, D), jnp.bfloat16)
        o_scr[S - 256:, :] = jnp.zeros((256, Dh), jnp.bfloat16)

        c = c_ref[...].astype(jnp.float32)
        sc = c * jax.nn.sigmoid(c)
        scb = jnp.broadcast_to(sc, (16, D)).astype(jnp.bfloat16)
        wm1_copy.wait()
        mod1 = jnp.dot(scb, wm_v[:, 0:2 * D], preferred_element_type=jnp.float32)
        mod_scr[:, 0:2 * D] = mod1[0:8]
        sa = mod_scr[0:1, 0:D]
        ca = mod_scr[0:1, D:2 * D]

        for i in range(nxc):
            x_copy(i).wait()
            r = slice(i * XC, (i + 1) * XC)
            xf = x_v[r, :].astype(jnp.float32)
            h_scr[r, :] = (_ln(xf) * (1.0 + ca) + sa).astype(jnp.bfloat16)

        scale = Dh ** -0.5 * LOG2E
        ztk = pl.multiple_of(z_ref[0], 8)
        sb = lambda u, g: sbs[(u % 2) * 4 + g]

        def red(x, op):
            n = x.shape[0] // 8
            return _tree([x[8 * i:8 * (i + 1), :] for i in range(n)], op)

        def qproj(i, wslot):
            r = slice(i * 256, (i + 1) * 256)
            q = jnp.dot(h_scr[r, :], wq_v[wslot], preferred_element_type=jnp.float32)
            q_scr[r, :] = (q * scale).astype(jnp.bfloat16)

        def oproj(i, wslot):
            r = slice(i * 256, (i + 1) * 256)
            acc_scr[r, :] += jnp.dot(o_scr[r, :], wo_v[wslot], preferred_element_type=jnp.float32)

        class St:
            pass

        def new_state():
            st = St()
            st.mx = {}
            st.atok = {}
            st.ls = {}
            st.accs = {}
            return st

        def a_chunk(st, n, kslot):
            u, c_ = divmod(n, 4)
            ul = u % nu
            qt = q_scr[ul * bq:(ul + 1) * bq, :]
            parts = []
            for m in range(4):
                r0 = 512 * c_ + 128 * m
                kk = k_v[kslot, r0:r0 + 128, :]
                s = _dot_t(kk, qt)
                sb(u, c_)[128 * m:128 * (m + 1), :] = s
                if m == 3:
                    st.atok[n] = s[tok_row:tok_row + 8, :]
                parts.append(red(s, jnp.maximum))
            sm = _tree(parts, jnp.maximum)
            st.mx[u] = sm if c_ == 0 else jnp.maximum(st.mx[u], sm)
            if c_ == 3:
                st.mx[u] = jnp.broadcast_to(jnp.max(st.mx[u], axis=0, keepdims=True), (8, bq))

        def exp_group(st, n, tok):
            u, g = divmod(n, 4)
            if tok is not None:
                sb(u, g)[pl.ds(ztk + 512, 8), :] = tok
            s = sb(u, g)[0:512, :]
            p = jnp.exp2(s - jnp.tile(st.mx[u], (64, 1)))
            ps = red(p, jnp.add)
            st.ls[u] = ps if g == 0 else st.ls[u] + ps
            return p.astype(jnp.bfloat16)

        def finish(acc, l, u):
            lsum = jnp.sum(l, axis=0, keepdims=True)
            o = acc * (1.0 / lsum)
            o_scr[u * bq:(u + 1) * bq, :] = o.T.astype(jnp.bfloat16)

        def pv(st, n, pb):
            u, g = divmod(n, 4)
            o = jnp.dot(vt_scr[:, 512 * g:512 * (g + 1)], pb, preferred_element_type=jnp.float32)
            st.accs[u] = o if g == 0 else st.accs[u] + o
            if g == 3:
                if u == nu - 1 and defer_finish:
                    oacc_scr[...] = st.accs[u]
                    carry_scr[24:32, :] = st.ls[u]
                else:
                    finish(st.accs[u], st.ls[u], u)

        wq_copy(0, 0).wait()
        qproj(0, 0)
        k_copy(0, 0).wait()
        st = new_state()
        for n in range(AH):
            a_chunk(st, n, 0)
        p0 = exp_group(st, 0, st.atok[AH - 1])
        p_scr[...] = p0
        carry_scr[0:8, :] = st.mx[0]
        carry_scr[8:16, :] = st.mx[1]
        carry_scr[16:24, :] = st.ls[0]
        if defer_finish:
            oacc_scr[...] = jnp.zeros_like(oacc_scr)
            carry_scr[24:32, :] = jnp.ones((8, bq), jnp.float32)

        wm2_copy.start()
        wg_copy.start()
        wu_copy.start()
        wd_copy.start()

        def head_body(h, carry):
            s0 = h % 3
            s1 = (h + 1) % 3
            s2 = (h + 2) % 3
            k_copy(h + 1, s1).wait()
            wq_copy(h + 1, s1).wait()
            v_copy(h, s0).wait()
            wo_copy(h, s0).wait()
            k_copy(h + 2, s2).start()
            wq_copy(h + 2, s2).start()
            v_copy(h + 1, s1).start()
            wo_copy(h + 1, s1).start()

            st = new_state()
            st.mx[0] = carry_scr[0:8, :]
            st.mx[1] = carry_scr[8:16, :]
            st.ls[0] = carry_scr[16:24, :]
            pcur = p_scr[...]

            vt_scr[...] = v_v[s0].T
            if defer_finish:
                finish(oacc_scr[...], carry_scr[24:32, :], nu - 1)

            ptok = {}
            for n in range(NS):
                i = n // 8
                pnext = None
                for ch in order:
                    if ch == 'e':
                        tok = st.atok.get(n + AH - 1)
                        pnext = exp_group(st, n + 1, tok)
                    elif ch == 'a':
                        a_chunk(st, n + AH, s0 if n + AH < NS else s1)
                    elif ch == 'p':
                        pv(st, n, pcur)
                        ptok[n] = st.accs[n // 4][tok_row:tok_row + 8, :]
                    elif ch == 'j':
                        if n % 8 == ostep:
                            if i == 0:
                                oproj(7, s2)
                            else:
                                oproj(i - 1, s0)
                        if n % 8 == qstep:
                            if i < 7:
                                qproj(i + 1, s0)
                            else:
                                qproj(0, s1)
                pcur = pnext
            p_scr[...] = pcur
            carry_scr[0:8, :] = st.mx[nu]
            carry_scr[8:16, :] = st.mx[nu + 1]
            carry_scr[16:24, :] = st.ls[nu]
            return carry

        jax.lax.fori_loop(0, NH, head_body, 0)

        k_copy(NH + 1, (NH + 1) % 3).wait()
        wq_copy(NH + 1, (NH + 1) % 3).wait()
        v_copy(NH, NH % 3).wait()
        wo_copy(NH, NH % 3).wait()

        if defer_finish:
            finish(oacc_scr[...], carry_scr[24:32, :], nu - 1)
        oproj(7, (NH - 1) % 3)

        wm2_copy.wait()
        mod2 = jnp.dot(scb, wm_v[:, 2 * D:6 * D], preferred_element_type=jnp.float32)
        mod_scr[:, 2 * D:6 * D] = mod2[0:8]
        ga = mod_scr[0:1, 2 * D:3 * D]
        sb_ = mod_scr[0:1, 3 * D:4 * D]
        cb = mod_scr[0:1, 4 * D:5 * D]
        gb = mod_scr[0:1, 5 * D:6 * D]
        wg_copy.wait()
        wu_copy.wait()
        wd_copy.wait()

        nfb = S // ffn_bm

        def pre(i):
            r = pl.ds(pl.multiple_of(i * ffn_bm, ffn_bm), ffn_bm)
            x1 = x_v[r, :].astype(jnp.float32) + ga * acc_scr[r, :]
            return (_ln(x1) * (1.0 + cb) + sb_).astype(jnp.bfloat16)

        def body(i, h2):
            r = pl.ds(pl.multiple_of(i * ffn_bm, ffn_bm), ffn_bm)
            g = jnp.dot(h2, wg_v[...], preferred_element_type=jnp.float32)
            u = jnp.dot(h2, wu_v[...], preferred_element_type=jnp.float32)
            a = (_gelu(g) * u).astype(jnp.bfloat16)
            y = jnp.dot(a, wd_v[...], preferred_element_type=jnp.float32)
            h2n = pre(jnp.minimum(i + 1, nfb - 1))
            x1 = x_v[r, :].astype(jnp.float32) + ga * acc_scr[r, :]
            out_v[r, :] = (x1 + gb * y).astype(out_v.dtype)
            out_copy(i).start()
            return h2n
        jax.lax.fori_loop(0, nfb, body, pre(0))
        for i in range(S // ffn_bm):
            out_copy(i).wait()

    @jax.jit
    def run(A_x, A_k_cache, A_v_cache, A_wq, A_wo, B_x, B_w_gate, B_w_up, B_w_down, c, w_mod):
        B, S, D = A_x.shape
        _, H, Sk, Dh = A_k_cache.shape
        F = B_w_gate.shape[1]
        x = A_x.reshape(S, D)
        k = A_k_cache.reshape(H, Sk, Dh)
        v = A_v_cache.reshape(H, Sk, Dh)
        z = jnp.asarray(np.zeros((8,), np.int32))
        anys = pl.BlockSpec(memory_space=pl.ANY)
        out = pl.pallas_call(
            kernel,
            in_specs=[
                pl.BlockSpec(memory_space=pltpu.SMEM),
                pl.BlockSpec(memory_space=pltpu.VMEM),
            ] + [anys] * 9,
            out_specs=anys,
            out_shape=jax.ShapeDtypeStruct((S, D), jnp.bfloat16),
            scratch_shapes=[
                pltpu.VMEM((S, D), jnp.bfloat16),
                pltpu.VMEM((S, D), jnp.bfloat16),
                pltpu.VMEM((8, 6 * D), jnp.float32),
                pltpu.VMEM((S, D), jnp.float32),
                pltpu.VMEM((S, Dh), jnp.bfloat16),
                pltpu.VMEM((Dh, Sk), jnp.bfloat16),
                pltpu.VMEM((S, Dh), jnp.bfloat16),
                pltpu.VMEM((512, bq), jnp.bfloat16),
                pltpu.VMEM((32, bq), jnp.float32),
                pltpu.VMEM((Dh, bq), jnp.float32),
                pltpu.VMEM((3, Sk, Dh), jnp.bfloat16),
                pltpu.VMEM((3, Sk, Dh), jnp.bfloat16),
                pltpu.VMEM((3, D, Dh), jnp.bfloat16),
                pltpu.VMEM((3, Dh, D), jnp.bfloat16),
                pltpu.VMEM((D, F), jnp.bfloat16),
                pltpu.VMEM((D, F), jnp.bfloat16),
                pltpu.VMEM((F, D), jnp.bfloat16),
                pltpu.VMEM((D, 6 * D), jnp.bfloat16),
                pltpu.VMEM((S, D), jnp.bfloat16),
                pltpu.SemaphoreType.DMA((3,)),
                pltpu.SemaphoreType.DMA((3,)),
                pltpu.SemaphoreType.DMA((3,)),
                pltpu.SemaphoreType.DMA((3,)),
                pltpu.SemaphoreType.DMA((S // 256,)),
                pltpu.SemaphoreType.DMA((2,)),
                pltpu.SemaphoreType.DMA((3,)),
                pltpu.SemaphoreType.DMA((S // ffn_bm,)),
            ] + [pltpu.VMEM((520, bq), jnp.float32) for _ in range(8)],
            compiler_params=pltpu.CompilerParams(
                vmem_limit_bytes=100 * 1024 * 1024, flags=flags,
            ),
        )(z, c, x, k, v, A_wq, A_wo, B_w_gate, B_w_up, B_w_down, w_mod)
        return out.reshape(B, S, D)
    return run


_run = _make()


def pallas_adaLN_cond__mha_block_cached__geglu_ffn__prompt_kernel(
    A_x, A_k_cache, A_v_cache, A_wq, A_wo, B_x, B_w_gate, B_w_up, B_w_down, c, w_mod,
):
    return _run(A_x, A_k_cache, A_v_cache, A_wq, A_wo, B_x,
                B_w_gate, B_w_up, B_w_down, c, w_mod)
```
